```python
import os as _os
_os.environ.setdefault("JAX_PLATFORMS", "cpu")
import jax
import jax.numpy as jnp

def _softmax(x, axis=-1):
    return jax.nn.softmax(x, axis=axis)
def _gelu(x):
    return jax.nn.gelu(x, approximate=True)
def _silu(x):
    return jax.nn.silu(x)
def _sigmoid(x):
    return jax.nn.sigmoid(x)
def _layernorm(x, axis=-1, eps=1e-5):
    m = jnp.mean(x, axis=axis, keepdims=True)
    v = jnp.var(x, axis=axis, keepdims=True)
    return (x - m) / jnp.sqrt(v + eps)
def _scatter_add(tgt, idx, src, axis=0):
    return tgt.at[idx].add(src)
def _segment_sum(src, seg, n):
    return jax.ops.segment_sum(src, seg, n)
class _Rng:
    def __init__(self, key):
        self._k = key
    def _next(self):
        self._k, sub = jax.random.split(self._k)
        return sub
    def normal(self, shape):
        return jax.random.normal(self._next(), shape, dtype=jnp.bfloat16)
    def randint(self, lo, hi, shape):
        return jax.random.randint(self._next(), shape, lo, hi, dtype=jnp.int32)
    def uniform(self, shape, lo=0.0, hi=1.0):
        return jax.random.uniform(self._next(), shape, jnp.bfloat16, lo, hi)
    def permutation(self, n):
        return jax.random.permutation(self._next(), n)


kernel_name = 'standalone__dcn_v2_cross__recsys'

def setup_inputs():
    _rng = _Rng(jax.random.key(int.from_bytes(__import__("os").urandom(4), "little")))
    _w = (lambda a: (lambda t: t.astype(jnp.bfloat16) if jnp.issubdtype(t.dtype, jnp.floating) else t)(jnp.asarray(a)))
    B, F, D, L = 4096, 26, 128, 6
    Din = min(F * D, 1024)
    return {
        "x0": _w((lambda *s: _rng.normal(s) * 0.05)(B, Din)),
        "ws": _w((lambda *s: _rng.normal(s) * 0.05)(L, Din, Din)),
        "bs": _w((lambda *s: _rng.normal(s) * 0.05)(L, Din)),
    }

def reference(x0, ws, bs):
    x = x0
    for l in range(ws.shape[0]):
        x = x0 * (x @ ws[l] + bs[l]) + x
    return x
```

```python
import jax
import jax.numpy as jnp
import jax.experimental.pallas as pl
import jax.experimental.pallas.tpu as pltpu

BM = 512
NC = 512
OSUB = 128


def _kernel(x_hbm, w_hbm, b_ref, o_hbm, xv, wv, ov, xa, xb, bf, sx, sw, so):
    L, D, _ = w_hbm.shape
    B = x_hbm.shape[0]
    nn = D // NC
    cp = pltpu.make_async_copy

    step = -(-(B - BM) // ((L - 1) * 128)) * 128
    edges = [min(BM + k * step, B) for k in range(L)]
    x_first = cp(x_hbm.at[:BM], xv.at[:BM], sx.at[0])
    x_rest = [
        cp(x_hbm.at[lo:hi], xv.at[lo:hi], sx.at[1 + k])
        for k, (lo, hi) in enumerate(zip(edges[:-1], edges[1:]))
    ]

    def w_first(n):
        c = slice(n * NC, (n + 1) * NC)
        return cp(w_hbm.at[0, :, c], wv.at[0, :, c], sw.at[n])

    def w_layer(l):
        return cp(w_hbm.at[l], wv.at[l], sw.at[nn + l - 1])

    def layer(l, x0, src, dst, c=slice(None)):
        y = jnp.dot(src[...], wv[l, :, c], preferred_element_type=jnp.float32)
        y = x0[:, c].astype(jnp.float32) * (y + bf[pl.ds(l, 1), c])
        dst[:, c] = (y + src[:, c].astype(jnp.float32)).astype(dst.dtype)

    x_first.start()
    for n in range(nn):
        w_first(n).start()
    bf[...] = b_ref[...].astype(jnp.float32)
    x_first.wait()
    x0, o = xv.at[:BM], ov.at[:BM]
    for n in range(nn):
        w_first(n).wait()
        if n == 0:
            w_layer(1).start()
        layer(0, x0, x0, o, slice(n * NC, (n + 1) * NC))

    def first_tile_layer(l, _):
        w_layer(l).wait()

        @pl.when(l + 1 < L)
        def _():
            w_layer(l + 1).start()

        for k, c in enumerate(x_rest):
            pl.when(l == k + 1)(c.start)
        xa[...] = o[...]
        layer(l, x0, xa, o)

    jax.lax.fori_loop(1, L, first_tile_layer, None)
    cp(o, o_hbm.at[:BM], so).start()
    for c in x_rest:
        c.wait()

    def tile(t, _):
        r0 = pl.multiple_of(t * BM, BM)
        x0 = src = xv.at[pl.ds(r0, BM)]
        for l in range(L - 1):
            dst = xb if l % 2 else xa
            layer(l, x0, src, dst)
            src = dst
        for s in range(BM // OSUB):
            r = pl.ds(pl.multiple_of(r0 + s * OSUB, OSUB), OSUB)
            layer(L - 1, xv.at[r], src.at[s * OSUB:(s + 1) * OSUB], ov.at[r])
            cp(ov.at[r], o_hbm.at[r], so).start()

    jax.lax.fori_loop(1, B // BM, tile, None)
    cp(ov, o_hbm, so).wait()


@jax.jit
def pallas_standalone__dcn_v2_cross__recsys_kernel(
    x0: jax.Array,
    ws: jax.Array,
    bs: jax.Array,
):
    B, D = x0.shape
    L = ws.shape[0]
    assert B % BM == 0 and D % NC == 0 and L >= 2
    hbm = pl.BlockSpec(memory_space=pl.ANY)
    return pl.pallas_call(
        _kernel,
        in_specs=[hbm, hbm, pl.BlockSpec(memory_space=pltpu.VMEM)],
        out_specs=hbm,
        out_shape=jax.ShapeDtypeStruct((B, D), x0.dtype),
        scratch_shapes=[
            pltpu.VMEM((B, D), x0.dtype),
            pltpu.VMEM(ws.shape, ws.dtype),
            pltpu.VMEM((B, D), x0.dtype),
            pltpu.VMEM((BM, D), x0.dtype),
            pltpu.VMEM((BM, D), x0.dtype),
            pltpu.VMEM(bs.shape, jnp.float32),
            pltpu.SemaphoreType.DMA((L,)),
            pltpu.SemaphoreType.DMA((D // NC + L - 1,)),
            pltpu.SemaphoreType.DMA(()),
        ],
        compiler_params=pltpu.CompilerParams(vmem_limit_bytes=64 * 2**20),
    )(x0, ws, bs)
```

```python
import jax
import jax.numpy as jnp
import jax.experimental.pallas as pl
import jax.experimental.pallas.tpu as pltpu

BM = 512
OSUB = 128


def _kernel(x_hbm, w_hbm, b_hbm, o_hbm, xv, wv, ov, xa, xb, bv, bf, s0, sx, sw, so):
    L, D, _ = w_hbm.shape
    B = x_hbm.shape[0]
    cp = pltpu.make_async_copy

    step = -(-(B - BM) // ((L - 1) * 128)) * 128
    edges = [min(BM + k * step, B) for k in range(L)]
    x_rest = [
        cp(x_hbm.at[lo:hi], xv.at[lo:hi], sx.at[k])
        for k, (lo, hi) in enumerate(zip(edges[:-1], edges[1:]))
    ]

    def w_layer(l):
        return cp(w_hbm.at[l], wv.at[l], sw.at[l - 1])

    def layer(l, x0, src, dst, c=slice(None)):
        y = jnp.dot(src[...], wv[l, :, c], preferred_element_type=jnp.float32)
        y = x0[:, c].astype(jnp.float32) * (y + bf[pl.ds(l, 1), c])
        dst[:, c] = (y + src[:, c].astype(jnp.float32)).astype(dst.dtype)

    ra, rb, rall = slice(0, BM // 2), slice(BM // 2, BM), slice(0, BM)
    ca, cb, cc = slice(0, D // 4), slice(D // 4, D // 2), slice(D // 2, D)
    bias = cp(b_hbm, bv, s0.at[0])
    x_a, x_b = (cp(x_hbm.at[r], xv.at[r], s0.at[1 + k])
                for k, r in enumerate((ra, rb)))
    w_a, w_b, w_c = (cp(w_hbm.at[0, :, c], wv.at[0, :, c], s0.at[3 + k])
                     for k, c in enumerate((ca, cb, cc)))
    for c in (bias, x_a, w_a, x_b):
        c.start()
    bias.wait()
    bf[...] = bv[...].astype(jnp.float32)
    x_a.wait()
    for rows, cols, needed, ahead in (
        (ra, ca, w_a, w_b),
        (rb, ca, x_b, w_c),
        (rall, cb, w_b, w_layer(1)),
        (rall, cc, w_c, None),
    ):
        needed.wait()
        if ahead is not None:
            ahead.start()
        layer(0, xv.at[rows], xv.at[rows], ov.at[rows], cols)

    x0, o = xv.at[:BM], ov.at[:BM]

    def first_tile_layer(l, _):
        w_layer(l).wait()

        @pl.when(l + 1 < L)
        def _():
            w_layer(l + 1).start()

        for k, c in enumerate(x_rest):
            pl.when(l == k + 1)(c.start)
        layer(l, x0, o, o)

    jax.lax.fori_loop(1, L, first_tile_layer, None)
    cp(o, o_hbm.at[:BM], so).start()
    for c in x_rest:
        c.wait()

    def tile(t, _):
        r0 = pl.multiple_of(t * BM, BM)
        x0 = src = xv.at[pl.ds(r0, BM)]
        for l in range(L - 1):
            dst = xb if l % 2 else xa
            layer(l, x0, src, dst)
            src = dst
        for s in range(BM // OSUB):
            r = pl.ds(pl.multiple_of(r0 + s * OSUB, OSUB), OSUB)
            layer(L - 1, xv.at[r], src.at[s * OSUB:(s + 1) * OSUB], ov.at[r])
            cp(ov.at[r], o_hbm.at[r], so).start()

    jax.lax.fori_loop(1, B // BM, tile, None)
    cp(ov, o_hbm, so).wait()


@jax.jit
def pallas_standalone__dcn_v2_cross__recsys_kernel(
    x0: jax.Array,
    ws: jax.Array,
    bs: jax.Array,
):
    B, D = x0.shape
    L = ws.shape[0]
    assert B % BM == 0 and D % 512 == 0 and L >= 2
    hbm = pl.BlockSpec(memory_space=pl.ANY)
    return pl.pallas_call(
        _kernel,
        in_specs=[hbm, hbm, hbm],
        out_specs=hbm,
        out_shape=jax.ShapeDtypeStruct((B, D), x0.dtype),
        scratch_shapes=[
            pltpu.VMEM((B, D), x0.dtype),
            pltpu.VMEM(ws.shape, ws.dtype),
            pltpu.VMEM((B, D), x0.dtype),
            pltpu.VMEM((BM, D), x0.dtype),
            pltpu.VMEM((BM, D), x0.dtype),
            pltpu.VMEM(bs.shape, bs.dtype),
            pltpu.VMEM(bs.shape, jnp.float32),
            pltpu.SemaphoreType.DMA((6,)),
            pltpu.SemaphoreType.DMA((L - 1,)),
            pltpu.SemaphoreType.DMA((L - 1,)),
            pltpu.SemaphoreType.DMA(()),
        ],
        compiler_params=pltpu.CompilerParams(vmem_limit_bytes=64 * 2**20),
    )(x0, ws, bs)
```
